```python
import os as _os
_os.environ.setdefault("JAX_PLATFORMS", "cpu")
import jax
import jax.numpy as jnp

def _softmax(x, axis=-1):
    return jax.nn.softmax(x, axis=axis)
def _gelu(x):
    return jax.nn.gelu(x, approximate=True)
def _silu(x):
    return jax.nn.silu(x)
def _sigmoid(x):
    return jax.nn.sigmoid(x)
def _layernorm(x, axis=-1, eps=1e-5):
    m = jnp.mean(x, axis=axis, keepdims=True)
    v = jnp.var(x, axis=axis, keepdims=True)
    return (x - m) / jnp.sqrt(v + eps)
def _scatter_add(tgt, idx, src, axis=0):
    return tgt.at[idx].add(src)
def _segment_sum(src, seg, n):
    return jax.ops.segment_sum(src, seg, n)
class _Rng:
    def __init__(self, key):
        self._k = key
    def _next(self):
        self._k, sub = jax.random.split(self._k)
        return sub
    def normal(self, shape):
        return jax.random.normal(self._next(), shape, dtype=jnp.bfloat16)
    def randint(self, lo, hi, shape):
        return jax.random.randint(self._next(), shape, lo, hi, dtype=jnp.int32)
    def uniform(self, shape, lo=0.0, hi=1.0):
        return jax.random.uniform(self._next(), shape, jnp.bfloat16, lo, hi)
    def permutation(self, n):
        return jax.random.permutation(self._next(), n)


kernel_name = 'interleave_layers__linear_kernel_hedgehog__ssm_conv_s4__prompt'

def setup_inputs():
    _rng = _Rng(jax.random.key(int.from_bytes(__import__("os").urandom(4), "little")))
    _w = (lambda a: (lambda t: t.astype(jnp.bfloat16) if jnp.issubdtype(t.dtype, jnp.floating) else t)(jnp.asarray(a)))
    def _A_setup():
        B, S, D, H = 1, 2048, 512, 32
        Dh = D // H
        return {
            "x": _w((lambda *s: _rng.normal(s) * 0.05)(B, S, D)),
            "wqkv": _w((lambda *s: _rng.normal(s) * 0.4)(D, 3 * D)),
            "w_phi": _w((lambda *s: _rng.normal(s) * 0.4)(H, Dh, Dh) * (Dh ** -0.5)),
            "wo": _w((lambda *s: _rng.normal(s) * 0.05)(D, D)),
        }
    _A_in = _A_setup()

    def _B_setup():
        B, L, D, N = 1, 2048, 512, 128
        A_re = -jnp.exp((lambda *s: _rng.normal(s) * 0.2)(D, N))
        A_im = jnp.pi * (lambda *s: _rng.normal(s) * 0.2)(D, N)
        B_re = (lambda *s: _rng.normal(s) * 0.2)(D, N)
        B_im = (lambda *s: _rng.normal(s) * 0.2)(D, N)
        C_re = (lambda *s: _rng.normal(s) * 0.2)(D, N)
        C_im = (lambda *s: _rng.normal(s) * 0.2)(D, N)
        log_dt = (lambda *s: _rng.normal(s) * 0.2)(D) * 0.5 - 4.0
        Dskip = (lambda *s: _rng.normal(s) * 0.2)(D)
        return {
            "u": _w((lambda *s: _rng.normal(s) * 0.05)(B, L, D)),
            "A_re": _w(A_re),
            "A_im": _w(A_im),
            "B_re": _w(B_re),
            "B_im": _w(B_im),
            "C_re": _w(C_re),
            "C_im": _w(C_im),
            "log_dt": _w(log_dt),
            "Dskip": _w(Dskip),
        }
    _B_in = _B_setup()

    return {
        "A_x": _A_in["x"],
        "A_wqkv": _A_in["wqkv"],
        "A_w_phi": _A_in["w_phi"],
        "A_wo": _A_in["wo"],
        "B_u": _B_in["u"],
        "B_A_re": _B_in["A_re"],
        "B_A_im": _B_in["A_im"],
        "B_B_re": _B_in["B_re"],
        "B_B_im": _B_in["B_im"],
        "B_C_re": _B_in["C_re"],
        "B_C_im": _B_in["C_im"],
        "B_log_dt": _B_in["log_dt"],
        "B_Dskip": _B_in["Dskip"],
    }

def reference(A_x, A_wqkv, A_w_phi, A_wo, B_u, B_A_re, B_A_im, B_B_re, B_B_im, B_C_re, B_C_im, B_log_dt, B_Dskip):
    def _A_ref(x, wqkv, w_phi, wo):
        B, S, D = x.shape
        H = 32; Dh = D // H
        qkv = (lambda x, *d: x.transpose(*d))((x @ wqkv).reshape(B, S, 3, H, Dh), 2, 0, 3, 1, 4)
        q, k, v = qkv[0], qkv[1], qkv[2]
        pq = jnp.einsum("bhsd,hdf->bhsf", q, w_phi)
        pk = jnp.einsum("bhsd,hdf->bhsf", k, w_phi)
        phi_q = jnp.concatenate([_softmax(pq, axis=-1), _softmax(-pq, axis=-1)], axis=-1)
        phi_k = jnp.concatenate([_softmax(pk, axis=-1), _softmax(-pk, axis=-1)], axis=-1)
        kv = jnp.einsum("bhsf,bhsd->bhfd", phi_k, v)
        z  = jnp.einsum("bhsf->bhf", phi_k)
        num = jnp.einsum("bhqf,bhfd->bhqd", phi_q, kv)
        den = jnp.einsum("bhqf,bhf->bhq", phi_q, z)[..., None] + 1e-6
        o = num / den
        return (lambda x, *d: x.transpose(*d))(o, 0, 2, 1, 3).reshape(B, S, D) @ wo

    def _B_ref(u, A_re, A_im, B_re, B_im, C_re, C_im, log_dt, Dskip):
        Bsz, L, D = u.shape
        dt = jnp.exp(log_dt)[:, None]
        A = A_re + 1j * A_im
        Bc = B_re + 1j * B_im
        Cc = C_re + 1j * C_im
        logdA = dt * A
        dB = dt * Bc
        l = (lambda x, dt: x.astype(dt))(jnp.arange(L), A_re.dtype)
        P = jnp.exp(logdA[:, :, None] * l[None, None, :])
        K = jnp.einsum("dn,dnl,dn->dl", Cc, P, dB).real
        L2 = 2 * L
        Kp = jnp.pad(K, ((0, 0), (0, L)))
        up = (lambda x, *d: x.transpose(*d))(u, 0, 2, 1)
        up = jnp.pad(up, ((0, 0), (0, 0), (0, L)))
        Kf = (lambda x, axes=(-2,-1): jnp.fft.rfft2(x.astype(jnp.float32), axes=axes))(Kp[:, None, :], axes=(-2, -1))
        Uf = (lambda x, axes=(-2,-1): jnp.fft.rfft2(x.astype(jnp.float32), axes=axes))(up[:, :, None, :], axes=(-2, -1))
        Yf = Uf * Kf[None, :, :, :]
        y = (lambda x, s, axes=(-2,-1): jnp.fft.irfft2(x, s=s, axes=axes).astype(jnp.bfloat16))(Yf, (1, L2), axes=(-2, -1))[:, :, 0, :L]
        y = (lambda x, *d: x.transpose(*d))(y, 0, 2, 1) + u * Dskip[None, None, :]
        return y

    x = A_x
    x = x + _A_ref(_layernorm(x, axis=-1), A_wqkv, A_w_phi, A_wo)
    x = x + _B_ref(_layernorm(x, axis=-1), B_A_re, B_A_im, B_B_re, B_B_im, B_C_re, B_C_im, B_log_dt, B_Dskip)
    x = x + _A_ref(_layernorm(x, axis=-1), A_wqkv, A_w_phi, A_wo)
    x = x + _B_ref(_layernorm(x, axis=-1), B_A_re, B_A_im, B_B_re, B_B_im, B_C_re, B_C_im, B_log_dt, B_Dskip)
    return x
```

```python
import functools
import numpy as np
import jax
import jax.numpy as jnp
from jax import lax
import jax.experimental.pallas as pl
import jax.experimental.pallas.tpu as pltpu

S = 2048
D = 512
C = 128
NC = S // C
TN = 256
NT = S // TN
LOG2E = 1.4426950408889634
F32 = jnp.float32
BF16 = jnp.bfloat16
U32 = jnp.uint32
TIE_LAG = False
MB = 64
TIE2 = 0
G1 = 8
UNR = 2
BC0 = 1
NQ = 4
FP = 129
P = 9


def _iota(shape, dim):
    return lax.broadcasted_iota(jnp.int32, shape, dim)


def _cmul(ar, ai, br, bi):
    return ar * br - ai * bi, ar * bi + ai * br


def _b(u):
    return pltpu.bitcast(u, BF16)


def _u(x):
    return pltpu.bitcast(x, U32)


def _pk(a, b):
    return pltpu.pack_elementwise([a, b], packed_dtype=BF16)


def _dot(a, b):
    return jnp.dot(a, b, preferred_element_type=F32)


def _dot_nt(a, b):
    return lax.dot_general(a, b, (((1,), (1,)), ((), ())), preferred_element_type=F32)


def _kernel(x_hbm, wqkv_hbm, wphi_hbm, wo_hbm, are_hbm, aim_hbm, bre_hbm, bim_hbm,
            cre_hbm, cim_hbm, ldt_ref, dsk_ref, o_hbm,
            x_ref, wqkv_ref, wo_ref, wphi_ref, prm_ref, sems, osems,
            xT, Wt, woT, phq, kvacc, Fc, Gc, K0, lam, l8, mu, cl, cc,
            dskb, UB, UR, p0, sb0, sb1, hb, yb0, yb1, yt0, yt1, xn0, xn1, zero_ref, *, phases):
    prm_copies = [pltpu.make_async_copy(h, prm_ref.at[i], sems.at[i])
                  for i, h in enumerate((are_hbm, aim_hbm, bre_hbm, bim_hbm, cre_hbm, cim_hbm))]
    w_copies = [pltpu.make_async_copy(wqkv_hbm, wqkv_ref, sems.at[6]),
                pltpu.make_async_copy(wo_hbm, wo_ref, sems.at[7]),
                pltpu.make_async_copy(wphi_hbm, wphi_ref, sems.at[12])]
    x_copies = [pltpu.make_async_copy(x_hbm.at[pl.ds(q * 512, 512)], x_ref.at[pl.ds(q * 512, 512)], sems.at[8 + q])
                for q in range(4)]
    for cp in prm_copies + w_copies + x_copies:
        cp.start()
    are_ref, aim_ref, bre_ref, bim_ref, cre_ref, cim_ref = (prm_ref.at[i] for i in range(6))

    def prep_weights():
        r = _iota((128, 128), 0)
        c = _iota((128, 128), 1)
        h8 = r // 16
        e = r % 16
        jj = c // 64
        f = (c % 64) // 4
        h4 = c % 4
        same_head = h8 == jj * 4 + h4
        pv = jnp.where(same_head & (e == f), 1.0, 0.0).astype(BF16)
        cc_ = _iota((32, 512), 1)
        sel = jnp.where(_iota((32, 512), 0) == (cc_ // 64) * 4 + cc_ % 4, 1.0, 0.0).astype(BF16)
        e1 = _dot(wphi_ref[...].reshape(256, 32), sel).reshape(16, 16, 512)
        fsel = _iota((16, 16, 512), 1) == (_iota((16, 16, 512), 2) % 64) // 4
        t1 = jnp.sum(jnp.where(fsel, e1, 0.0), axis=1)
        rho = (c % 64) // 2 + 32 * (c % 2)
        vrow = rho // 2 + 32 * (rho % 2)
        po = jnp.where((h8 == jj * 4 + vrow % 4) & (e == vrow // 4), 1.0, 0.0).astype(BF16)

        def kt(m):
            return _b(_pk(m[0:256], m[256:512])).T
        for b in range(4):
            wt = jnp.concatenate([t1[:, b * 128:(b + 1) * 128]] * 8, axis=0)
            pq = jnp.where(same_head, wt * LOG2E, 0.0).astype(BF16)
            qT = kt(_dot(wqkv_ref[:, b * 128:(b + 1) * 128], pq))
            kT = kt(_dot(wqkv_ref[:, 512 + b * 128:512 + (b + 1) * 128], pq))
            vT = kt(_dot(wqkv_ref[:, 1024 + b * 128:1024 + (b + 1) * 128], pv))
            for t in range(2):
                j = 2 * b + t
                Wt[j, 0:32, :] = _u(qT[t * 64:(t + 1) * 64])
                Wt[j, 32:64, :] = _u(kT[t * 64:(t + 1) * 64])
                Wt[j, 64:96, :] = _u(vT[t * 64:(t + 1) * 64])
            wob = wo_ref[b * 128:(b + 1) * 128, :].T
            wop = _dot(wob, po)
            woT[:, b * 128:(b + 1) * 128] = _u(wop.astype(BF16))

    def load_x_steps():
        def step(t0):
            def f():
                xT[:, t0:t0 + 128] = x_ref[t0:t0 + 128, :].T.astype(F32)
            return f
        return [step(128 * q) for q in range(16)]

    def sum8(a):
        return jnp.sum(a.reshape(a.shape[0] // 8, 8, a.shape[1]), axis=0)

    def ln_stat_steps(t0, st):
        steps = []

        def s1(b):
            def f():
                s = sum8(xT[b * 128:(b + 1) * 128, pl.ds(t0, TN)])
                st['a'] = s if b == 0 else st['a'] + s
                if b == 3:
                    st['m'] = jnp.sum(st['a'], axis=0, keepdims=True) * (1.0 / D)
                return _u32(st['a'][:, 0:128])
            return f

        def s2(b):
            def f():
                xc = xT[b * 64:(b + 1) * 64, pl.ds(t0, TN)] - st['m']
                s = sum8(xc * xc)
                st['a'] = s if b == 0 else st['a'] + s
                if b == 7:
                    st['rs'] = lax.rsqrt(jnp.sum(st['a'], axis=0, keepdims=True) * (1.0 / D) + 1e-5)
                return _u32(st['a'][:, 0:128])
            return f
        return [s1(b) for b in range(4)] + [s2(b) for b in range(8)]

    def ln_steps(xn_ref, t0):
        st = {}

        def s3(b):
            def f():
                xa = xT[b * 64:(b + 1) * 64, pl.ds(t0, TN)]
                xb = xT[256 + b * 64:256 + (b + 1) * 64, pl.ds(t0, TN)]
                w = _pk((xa - st['m']) * st['rs'], (xb - st['m']) * st['rs'])
                xn_ref[b * 64:(b + 1) * 64, :] = w
                return w[56:64, 128:256]
            return f
        return ln_stat_steps(t0, st) + [s3(b) for b in range(4)]

    def _u32(a):
        return pltpu.bitcast(a, U32)

    def run_all(steps):
        toks = []
        for s in steps:
            r = s()
            if r is not None:
                toks.append(r)
        return toks

    def tie(w, toks):
        if not toks:
            return w
        z = zero_ref[...]
        acc = None
        for tk in toks:
            a = tk & z
            acc = a if acc is None else acc | a
        top = jnp.concatenate([w[0:8, 0:128] | acc, w[0:8, 128:]], axis=1)
        return jnp.concatenate([top, w[8:]], axis=0)

    def spread(n_main, side):
        slots = [[] for _ in range(n_main)]
        for i, s in enumerate(side):
            slots[min(n_main - 1, (i * n_main) // max(1, len(side)))].append(s)
        return slots

    def halves(a):
        return pltpu.roll(a, 4, 0)

    def feat(p):
        p3 = p.reshape(8, 8, TN)
        mx = jnp.max(p3, axis=0)
        mn = jnp.min(p3, axis=0)
        mx = jnp.maximum(mx, halves(mx))
        mn = jnp.minimum(mn, halves(mn))
        ep = jnp.exp2(p3 - mx[None])
        en = jnp.exp2(mn[None] - p3)
        sp = jnp.sum(ep, axis=0)
        sn = jnp.sum(en, axis=0)
        sp = sp + halves(sp)
        sn = sn + halves(sn)
        rp = 1.0 / sp
        rn = 1.0 / sn
        ep = (ep * rp[None]).reshape(64, TN)
        en = (en * rn[None]).reshape(64, TN)
        return _pk(ep, en)

    def a_layer(extra1=None, extra2=None):
        kvacc[...] = jnp.zeros_like(kvacc)
        ones = jnp.full((8, TN), 0x3F803F80, U32)

        def p1_tile(t, xn_cur, xn_nxt):
            t0 = pl.multiple_of(t * TN, TN)

            def mm(j, part, toks=()):
                return _dot(_b(tie(Wt[j, 32 * part:32 * part + 32, :], toks)), _b(xn_cur[...]))
            seq = [(j, p) for j in range(8) for p in range(3)]
            tn0 = pl.multiple_of(jnp.minimum(t + 1, NT - 1) * TN, TN)
            side = ln_steps(xn_nxt, tn0)
            slots = spread(len(seq) - 2, side)
            if extra1 is not None:
                slots2 = spread(len(seq), extra1(t))
            cur = mm(0, 0)
            pk = None
            pend = []
            lag = [[], []]
            for idx, (j, p) in enumerate(seq):
                nxt = mm(*seq[idx + 1], lag[0]) if idx + 1 < len(seq) else None
                if p == 0:
                    phq[j, :, pl.ds(t0, TN)] = feat(cur)
                elif p == 1:
                    pk = feat(cur)
                else:
                    v1 = _b(jnp.concatenate([_pk(cur[0:32], cur[32:64]), ones], axis=0))
                    kvacc[j] += _dot_nt(v1, _b(pk))
                toks = []
                if idx < len(slots):
                    toks += run_all(slots[idx])
                if extra1 is not None:
                    toks += run_all(slots2[idx])
                lag = [lag[1], toks] if TIE_LAG else [toks, []]
                cur = nxt

        run_all(ln_steps(xn0, 0))

        def p1(i, carry):
            p1_tile(2 * i, xn0, xn1)
            p1_tile(2 * i + 1, xn1, xn0)
            return carry
        with jax.named_scope('A_p1'):
            lax.fori_loop(0, NT // 2, p1, 0)

        mask = ((_iota((80, 128), 0) // 2) % 4) == ((_iota((80, 128), 1) // 2) % 4)

        def o_steps(ob, t0):
            def nd(j):
                kvm = jnp.where(mask, kvacc[j], 0.0).astype(BF16)
                return _dot(kvm, _b(phq[j, :, pl.ds(t0, TN)]))
            st = {}

            def step(j):
                def f():
                    if j == 0:
                        st['cur'] = nd(0)
                    cur = st['cur']
                    if j < 7:
                        st['cur'] = nd(j + 1)
                    rden = 1.0 / (cur[64:72] + 1e-6)
                    o = (cur[0:64].reshape(8, 8, TN) * rden[None]).reshape(64, TN)
                    w = _pk(o[0:32], o[32:64])
                    ob[j * 32:(j + 1) * 32, :] = w
                    return w[24:32, 128:256]
                return f
            return [step(j) for j in range(8)]

        rev_idx = 127 - _iota((8, 128), 1)

        def lnb_steps(t, st):
            t0 = pl.multiple_of(t * TN, TN)

            def s3(b):
                def f():
                    xb = xT[b * 64:(b + 1) * 64, pl.ds(t0, TN)]
                    xn = (xb - st['m']) * st['rs']
                    dk = dskb[b * 64:(b + 1) * 64, :]
                    xT[b * 64:(b + 1) * 64, pl.ds(t0, TN)] = xb + xn * jnp.concatenate([dk, dk], axis=1)
                    w = _pk(xn[:, 0:128], xn[:, 128:256])
                    for r in range(8):
                        wr = w[r * 8:(r + 1) * 8]
                        UB[pl.ds((b * 64 + r * 8) * P + t, 8, stride=P), :] = wr
                        UR[pl.ds((b * 64 + r * 8) * P + t, 8, stride=P), :] = jnp.take_along_axis(wr, rev_idx, axis=1)
                    return w[56:64]
                return f
            return ln_stat_steps(t0, st)[4:] + [s3(b) for b in range(8)]

        def p2_tile(t, ob_cur, ob_nxt, st_prev):
            t0 = pl.multiple_of(t * TN, TN)
            tn0 = pl.multiple_of(jnp.minimum(t + 1, NT - 1) * TN, TN)
            nb = 512 // MB
            sideA = spread(nb, o_steps(ob_nxt, tn0))
            sideB = spread(nb, lnb_steps(t - 1, st_prev) if st_prev is not None else [])
            sideC = spread(nb, extra2(t) if extra2 is not None else [])

            def mm(b, toks=()):
                return _dot(_b(tie(woT[b * MB // 2:(b + 1) * MB // 2, :], toks)), _b(ob_cur[...]))
            cur = mm(0)
            a = None
            lag = [[], []]
            for b in range(nb):
                nxt = mm(b + 1, lag[0]) if b < nb - 1 else None
                xnew = xT[b * MB:(b + 1) * MB, pl.ds(t0, TN)] + cur
                xT[b * MB:(b + 1) * MB, pl.ds(t0, TN)] = xnew
                s = sum8(xnew)
                a = s if a is None else a + s
                toks = run_all(sideA[b]) + run_all(sideB[b]) + run_all(sideC[b])
                if TIE2 == 0:
                    toks = []
                lag = [lag[1], toks] if TIE2 == 2 else [toks, []]
                cur = nxt
            return jnp.sum(a, axis=0, keepdims=True) * (1.0 / D)

        run_all(o_steps(xn0, 0))
        m0 = p2_tile(0, xn0, xn1, None)
        m1 = p2_tile(1, xn1, xn0, {'m': m0})

        def p2(i, m):
            m = p2_tile(2 * i, xn0, xn1, {'m': m})
            return p2_tile(2 * i + 1, xn1, xn0, {'m': m})
        with jax.named_scope('A_p2loop'):
            m7 = lax.fori_loop(1, NT // 2, p2, m1)
        run_all(lnb_steps(NT - 1, {'m': m7}))

    def _interleave(a, b):
        return _b(pltpu.pack_elementwise([a, b], packed_dtype=BF16))

    def prep_ssm():
        ldt = jnp.broadcast_to(ldt_ref[...].astype(F32).reshape(1, D), (128, D)).T
        dt = jnp.exp(ldt).astype(BF16).astype(F32)
        dskb[...] = jnp.broadcast_to(dsk_ref[...].astype(F32).reshape(1, D), (128, D)).T
        lr = dt * are_ref[...].astype(F32)
        li = dt * aim_ref[...].astype(F32)
        m = jnp.exp(lr)
        l1r, l1i = m * jnp.cos(li), m * jnp.sin(li)
        lam[0] = l1r
        lam[1] = l1i
        a, b = l1r, l1i
        for k in range(7):
            a, b = a * a - b * b, 2.0 * a * b
            if k == 3:
                l8[0] = a
                l8[1] = b
        mu[0] = a
        mu[1] = b
        dbr = dt * bre_ref[...].astype(F32)
        dbi = dt * bim_ref[...].astype(F32)
        cr, ci = _cmul(cre_ref[...].astype(F32), cim_ref[...].astype(F32), dbr, dbi)
        cc[0] = cr
        cc[1] = ci
        a, b = _cmul(cr, ci, l1r, l1i)
        cl[0] = a
        cl[1] = b

    def bc(ref, i, d):
        if BC0:
            return ref[i, pl.ds(d, 8, stride=0), :]
        return jnp.broadcast_to(ref[i, pl.ds(d, 1), :], (8, 128))

    def gen_steps(g):
        g0 = pl.multiple_of(g * 8, 8)

        def base():
            ar = lam[0, pl.ds(g0, 8), :]
            ai = lam[1, pl.ds(g0, 8), :]
            ar, ai = ar * ar - ai * ai, 2.0 * ar * ai
            pr = jnp.ones((8, 128), F32)
            pi = jnp.zeros((8, 128), F32)
            for r in range(8):
                p0[0, pl.ds(r, 8, stride=P), :] = pr
                p0[1, pl.ds(r, 8, stride=P), :] = pi
                if r == 0:
                    pr, pi = ar, ai
                elif r < 7:
                    pr, pi = _cmul(pr, pi, ar, ai)
        def chan(d8):
            def f():
                d = g0 + d8
                br = bc(l8, 0, d)
                bi = bc(l8, 1, d)
                l1r = bc(lam, 0, d)
                l1i = bc(lam, 1, d)
                qr = p0[0, d8 * P:d8 * P + 8, :]
                qi = p0[1, d8 * P:d8 * P + 8, :]
                wr, wi = [], []
                for k in range(8):
                    if k > 0:
                        qr, qi = _cmul(qr, qi, br, bi)
                    orr, oi = _cmul(qr, qi, l1r, l1i)
                    wr.append(_pk(qr, orr))
                    wi.append(_pk(qi, oi))
                frw = jnp.concatenate(wr, axis=0)
                fiw = jnp.concatenate(wi, axis=0)
                Fc[d, 0:64, :] = frw
                Fc[d, 64:128, :] = fiw
                grb = _b(frw).T
                gib = _b(fiw).T
                Gc[d, 0:64, :] = _u(grb)
                Gc[d, 64:128, :] = _u(gib)
            return f
        return [base] + [chan(d8) for d8 in range(8)]

    def b_layer(first):
        rev_idx = 127 - _iota((8, 128), 1)
        tri = _iota((16, 128), 1) >= _iota((16, 128), 0)
        lane = _iota((8, 128), 1)

        def stage_i(g, sb):
            g0 = pl.multiple_of(g * 8, 8)
            for d8 in range(8):
                d = g0 + d8
                ur = _b(UR[pl.ds(d * P, 8), :])
                sr = _dot(ur, _b(Fc[d, 0:64, :]))
                si = _dot(ur, _b(Fc[d, 64:128, :]))
                for hf in range(2):
                    sb[0, pl.ds(8 * P * hf + d8, 8, stride=P), :] = sr[8 * hf:8 * hf + 8]
                    sb[1, pl.ds(8 * P * hf + d8, 8, stride=P), :] = si[8 * hf:8 * hf + 8]

        def stage_so(g, sb, yb):
            g0 = pl.multiple_of(g * 8, 8)
            mr = mu[0, pl.ds(g0, 8), :]
            mi = mu[1, pl.ds(g0, 8), :]
            cr = cl[0, pl.ds(g0, 8), :]
            ci = cl[1, pl.ds(g0, 8), :]
            zero = jnp.zeros((8, 128), F32)
            hr = hi = None
            prev = None
            for c in range(NC):
                if c == 0:
                    a, b = zero, zero
                else:
                    a, b = _cmul(cr, ci, hr, hi)
                    b = -b
                if c % 2 == 0:
                    prev = (a, b)
                else:
                    hb[0, pl.ds(c // 2, 8, stride=P), :] = pltpu.pack_elementwise([prev[0], a], packed_dtype=BF16)
                    hb[1, pl.ds(c // 2, 8, stride=P), :] = pltpu.pack_elementwise([prev[1], b], packed_dtype=BF16)
                if c < NC - 1:
                    sr = sb[0, c * P:c * P + 8, :]
                    si = sb[1, c * P:c * P + 8, :]
                    if c == 0:
                        hr, hi = sr, si
                    else:
                        a, b = _cmul(mr, mi, hr, hi)
                        hr, hi = a + sr, b + si
            for d8 in range(8):
                d = g0 + d8
                lr = hb[0, d8 * P:d8 * P + 8, :]
                li = hb[1, d8 * P:d8 * P + 8, :]
                if first:
                    cr = jnp.broadcast_to(cc[0, pl.ds(d, 1), :], (8, 128))
                    ci = jnp.broadcast_to(-cc[1, pl.ds(d, 1), :], (8, 128))
                    lr = jnp.concatenate([lr, _pk(cr, cr)], axis=0)
                    li = jnp.concatenate([li, _pk(ci, ci)], axis=0)
                y = _dot(_b(lr), _b(Gc[d, 0:64, :])) + _dot(_b(li), _b(Gc[d, 64:128, :]))
                if first:
                    K0[pl.ds(pl.multiple_of(d * 8, 8), 8), :] = y[16:24]
                for hf in range(2):
                    yb[pl.ds(8 * P * hf + d8, 8, stride=P), :] = y[8 * hf:8 * hf + 8]

        def stage_t(g, yt):
            g0 = pl.multiple_of(g * 8, 8)
            for d8 in range(8):
                d = g0 + d8
                k8 = K0[pl.ds(pl.multiple_of(d * 8, 8), 8), :]
                kb = jnp.concatenate([k8, k8], axis=0)
                b0 = _u(jnp.where(tri, pltpu.roll(kb, 0, 1, stride=1, stride_axis=0), 0.0).astype(BF16))
                rows = [b0]
                for k in range(1, 8):
                    rows.append(jnp.where(lane >= 16 * k, pltpu.roll(b0, 16 * k, 1), jnp.uint32(0)))
                y = _dot(_b(UB[pl.ds(d * P, 8), :]), _b(jnp.concatenate(rows, axis=0)))
                for hf in range(2):
                    yt[pl.ds(8 * P * hf + d8, 8, stride=P), :] = y[8 * hf:8 * hf + 8]

        def stage_x(g, yb, yt):
            g0 = pl.multiple_of(g * 8, 8)
            for c in range(NC):
                xT[pl.ds(g0, 8), c * C:(c + 1) * C] += yb[c * P:c * P + 8, :] + yt[c * P:c * P + 8, :]

        sbs, ybs, yts = (sb0, sb1), (yb0, yb1), (yt0, yt1)

        def step(g, par, do_i=True, do_x=True, do_t=True):
            if do_i:
                stage_i(g + 1, sbs[1 - par])
            if do_x:
                stage_x(g - 2, ybs[par], yts[par])
            stage_so(g, sbs[par], ybs[par])
            if do_t:
                stage_t(g - 1, yts[1 - par])

        stage_i(0, sb0)
        step(0, 0, do_x=False, do_t=False)
        step(1, 1, do_x=False)

        def grp(i, carry):
            for q in range(2 * UNR):
                step(2 + 2 * UNR * i + q, q % 2)
            return carry
        with jax.named_scope('B_loop%d' % first):
            lax.fori_loop(0, 60 // (2 * UNR), grp, 0)
        step(62, 0)
        step(63, 1, do_i=False)
        stage_t(63, yt1)
        stage_x(62, yb0, yt0)
        stage_x(63, yb1, yt1)

    def store_out():
        cps = []
        rows = S // NQ
        for q in range(NQ):
            for hf in range(rows // 128):
                t0 = q * rows + hf * 128
                x_ref[t0:t0 + 128, :] = xT[:, t0:t0 + 128].astype(BF16).T
            cp = pltpu.make_async_copy(x_ref.at[pl.ds(q * rows, rows)], o_hbm.at[pl.ds(q * rows, rows)], osems.at[q])
            cp.start()
            cps.append(cp)
        for cp in cps:
            cp.wait()

    zero_ref[...] = jnp.zeros((8, 128), U32)
    for cp in prm_copies:
        cp.wait()
    with jax.named_scope('prep_ssm'):
        prep_ssm()
    for cp in w_copies:
        cp.wait()
    with jax.named_scope('prep_w'):
        prep_weights()
    with jax.named_scope('load_x'):
        xs = load_x_steps()
        for q in range(4):
            x_copies[q].wait()
            for s_ in xs[4 * q:4 * q + 4]:
                s_()

    if 'g' in phases:
        def gb(g, carry):
            run_all(gen_steps(g))
            return carry
        lax.fori_loop(0, 64, gb, 0)
    nb_done = [0]
    for ph in phases:
        if ph == 'A':
            with jax.named_scope('A2'):
                a_layer()
        elif ph == 'G':
          with jax.named_scope('A1'):
            a_layer(lambda t: [s for q in range(G1) for s in gen_steps(t * G1 + q)],
                    lambda t: [s for q in range(8 - G1) for s in gen_steps(8 * G1 + t * (8 - G1) + q)])
        elif ph == 'B':
            with jax.named_scope('B%d' % nb_done[0]):
                b_layer(nb_done[0] == 0)
            nb_done[0] += 1
    with jax.named_scope('store'):
        store_out()


@jax.jit
def pallas_interleave_layers__linear_kernel_hedgehog__ssm_conv_s4__prompt_kernel(
        A_x, A_wqkv, A_w_phi, A_wo, B_u, B_A_re, B_A_im, B_B_re, B_B_im, B_C_re, B_C_im, B_log_dt, B_Dskip):
    del B_u
    x = A_x.reshape(S, D)
    V = pltpu.VMEM
    HBM = pl.BlockSpec(memory_space=pl.ANY)
    VM = pl.BlockSpec(memory_space=pltpu.VMEM)
    scratch = [
        V((S, D), BF16), V((D, 3 * D), BF16), V((D, D), BF16), V((16, 16, 32), BF16), V((6, D, 128), BF16),
        pltpu.SemaphoreType.DMA((13,)), pltpu.SemaphoreType.DMA((8,)),
        V((D, S), F32),
        V((8, 96, D), U32),
        V((D // 2, D), U32),
        V((8, 64, S), U32),
        V((8, 80, 128), F32),
        V((D, 128, 128), U32),
        V((D, 128, 128), U32),
        V((D * 8, 128), F32),
        V((2, D, 128), F32), V((2, D, 128), F32), V((2, D, 128), F32), V((2, D, 128), F32), V((2, D, 128), F32),
        V((D, 128), F32),
        V((D * P, 128), U32), V((D * P, 128), U32),
        V((2, 8 * P, 128), F32),
        V((2, NC * P, 128), F32), V((2, NC * P, 128), F32),
        V((2, 8 * P, 128), U32),
        V((NC * P, 128), F32), V((NC * P, 128), F32), V((NC * P, 128), F32), V((NC * P, 128), F32),
        V((D // 2, TN), U32), V((D // 2, TN), U32),
        V((8, 128), U32),
    ]
    out = pl.pallas_call(
        functools.partial(_kernel, phases='wpGBAB'),
        out_shape=jax.ShapeDtypeStruct((S, D), BF16),
        in_specs=[HBM, HBM, HBM, HBM, HBM, HBM, HBM, HBM, HBM, HBM, VM, VM],
        out_specs=HBM,
        scratch_shapes=scratch,
        compiler_params=pltpu.CompilerParams(vmem_limit_bytes=120 * 1024 * 1024),
    )(x, A_wqkv, jnp.transpose(A_w_phi, (1, 2, 0)), A_wo, B_A_re, B_A_im, B_B_re, B_B_im, B_C_re, B_C_im,
      B_log_dt, B_Dskip)
    return out.reshape(1, S, D)
```

```python
import functools
import jax
import jax.numpy as jnp
from jax import lax
import jax.experimental.pallas as pl
import jax.experimental.pallas.tpu as pltpu

S = 2048
D = 512
C = 128
NC = S // C
TN = 256
NT = S // TN
LOG2E = 1.4426950408889634
F32 = jnp.float32
BF16 = jnp.bfloat16
U32 = jnp.uint32
TIE_LAG = False
MB = 64
TIE2 = 0
G1 = 8
UNR = 2
P = 9


def _iota(shape, dim):
    return lax.broadcasted_iota(jnp.int32, shape, dim)


def _cmul(ar, ai, br, bi):
    return ar * br - ai * bi, ar * bi + ai * br


def _b(u):
    return pltpu.bitcast(u, BF16)


def _u(x):
    return pltpu.bitcast(x, U32)


def _pk(a, b):
    return pltpu.pack_elementwise([a, b], packed_dtype=BF16)


def _dot(a, b):
    return jnp.dot(a, b, preferred_element_type=F32)


def _dot_nt(a, b):
    return lax.dot_general(a, b, (((1,), (1,)), ((), ())), preferred_element_type=F32)


def _kernel(x_hbm, wqkv_hbm, wphi_hbm, wo_hbm, are_hbm, aim_hbm, bre_hbm, bim_hbm,
            cre_hbm, cim_hbm, ldt_ref, dsk_ref, o_hbm,
            x_ref, wqkv_ref, wo_ref, wphi_ref, prm_ref, ostg, sems, osems,
            xT, Wt, woT, phq, kvacc, Fc, Gc, Tc, K0, lam, l8, mu, cl, cc,
            dskb, UB, UR, p0, sb0, sb1, hb, yb0, yb1, yt0, yt1, xn0, xn1, zero_ref, *, phases):
    prm_copies = [pltpu.make_async_copy(h, prm_ref.at[i], sems.at[i])
                  for i, h in enumerate((are_hbm, aim_hbm, bre_hbm, bim_hbm, cre_hbm, cim_hbm))]
    w_copies = [pltpu.make_async_copy(wqkv_hbm, wqkv_ref, sems.at[6]),
                pltpu.make_async_copy(wo_hbm, wo_ref, sems.at[7]),
                pltpu.make_async_copy(wphi_hbm, wphi_ref, sems.at[12])]
    x_copies = [pltpu.make_async_copy(x_hbm.at[pl.ds(q * 512, 512)], x_ref.at[pl.ds(q * 512, 512)], sems.at[8 + q])
                for q in range(4)]
    for cp in prm_copies + w_copies + x_copies:
        cp.start()
    are_ref, aim_ref, bre_ref, bim_ref, cre_ref, cim_ref = (prm_ref.at[i] for i in range(6))

    def prep_weights():
        r = _iota((128, 128), 0)
        c = _iota((128, 128), 1)
        h8 = r // 16
        e = r % 16
        jj = c // 64
        f = (c % 64) // 4
        h4 = c % 4
        same_head = h8 == jj * 4 + h4
        pv = jnp.where(same_head & (e == f), 1.0, 0.0).astype(BF16)
        cc_ = _iota((32, 512), 1)
        sel = jnp.where(_iota((32, 512), 0) == (cc_ // 64) * 4 + cc_ % 4, 1.0, 0.0).astype(BF16)
        e1 = _dot(wphi_ref[...].reshape(256, 32), sel).reshape(16, 16, 512)
        fsel = _iota((16, 16, 512), 1) == (_iota((16, 16, 512), 2) % 64) // 4
        t1 = jnp.sum(jnp.where(fsel, e1, 0.0), axis=1)
        rho = (c % 64) // 2 + 32 * (c % 2)
        vrow = rho // 2 + 32 * (rho % 2)
        po = jnp.where((h8 == jj * 4 + vrow % 4) & (e == vrow // 4), 1.0, 0.0).astype(BF16)

        def kt(m):
            return _b(_pk(m[0:256], m[256:512])).T
        for b in range(4):
            wt = jnp.concatenate([t1[:, b * 128:(b + 1) * 128]] * 8, axis=0)
            pq = jnp.where(same_head, wt * LOG2E, 0.0).astype(BF16)
            qT = kt(_dot(wqkv_ref[:, b * 128:(b + 1) * 128], pq))
            kT = kt(_dot(wqkv_ref[:, 512 + b * 128:512 + (b + 1) * 128], pq))
            vT = kt(_dot(wqkv_ref[:, 1024 + b * 128:1024 + (b + 1) * 128], pv))
            for t in range(2):
                j = 2 * b + t
                Wt[j, 0:32, :] = _u(qT[t * 64:(t + 1) * 64])
                Wt[j, 32:64, :] = _u(kT[t * 64:(t + 1) * 64])
                Wt[j, 64:96, :] = _u(vT[t * 64:(t + 1) * 64])
            wob = wo_ref[b * 128:(b + 1) * 128, :].T
            wop = _dot(wob, po)
            woT[:, b * 128:(b + 1) * 128] = _u(wop.astype(BF16))

    def load_x_steps():
        def step(t0):
            def f():
                xT[:, t0:t0 + 128] = x_ref[t0:t0 + 128, :].T.astype(F32)
            return f
        return [step(128 * q) for q in range(16)]

    def sum8(a):
        return jnp.sum(a.reshape(a.shape[0] // 8, 8, a.shape[1]), axis=0)

    def ln_stat_steps(t0, st):
        steps = []

        def s1(b):
            def f():
                s = sum8(xT[b * 128:(b + 1) * 128, pl.ds(t0, TN)])
                st['a'] = s if b == 0 else st['a'] + s
                if b == 3:
                    st['m'] = jnp.sum(st['a'], axis=0, keepdims=True) * (1.0 / D)
                return _u32(st['a'][:, 0:128])
            return f

        def s2(b):
            def f():
                xc = xT[b * 64:(b + 1) * 64, pl.ds(t0, TN)] - st['m']
                s = sum8(xc * xc)
                st['a'] = s if b == 0 else st['a'] + s
                if b == 7:
                    st['rs'] = lax.rsqrt(jnp.sum(st['a'], axis=0, keepdims=True) * (1.0 / D) + 1e-5)
                return _u32(st['a'][:, 0:128])
            return f
        return [s1(b) for b in range(4)] + [s2(b) for b in range(8)]

    def ln_steps(xn_ref, t0):
        st = {}

        def s3(b):
            def f():
                xa = xT[b * 64:(b + 1) * 64, pl.ds(t0, TN)]
                xb = xT[256 + b * 64:256 + (b + 1) * 64, pl.ds(t0, TN)]
                w = _pk((xa - st['m']) * st['rs'], (xb - st['m']) * st['rs'])
                xn_ref[b * 64:(b + 1) * 64, :] = w
                return w[56:64, 128:256]
            return f
        return ln_stat_steps(t0, st) + [s3(b) for b in range(4)]

    def _u32(a):
        return pltpu.bitcast(a, U32)

    def run_all(steps):
        toks = []
        for s in steps:
            r = s()
            if r is not None:
                toks.append(r)
        return toks

    def tie(w, toks):
        if not toks:
            return w
        z = zero_ref[...]
        acc = None
        for tk in toks:
            a = tk & z
            acc = a if acc is None else acc | a
        top = jnp.concatenate([w[0:8, 0:128] | acc, w[0:8, 128:]], axis=1)
        return jnp.concatenate([top, w[8:]], axis=0)

    def spread(n_main, side):
        slots = [[] for _ in range(n_main)]
        for i, s in enumerate(side):
            slots[min(n_main - 1, (i * n_main) // max(1, len(side)))].append(s)
        return slots

    def halves(a):
        return pltpu.roll(a, 4, 0)

    def feat(p):
        p3 = p.reshape(8, 8, TN)
        mx = jnp.max(p3, axis=0)
        mn = jnp.min(p3, axis=0)
        mx = jnp.maximum(mx, halves(mx))
        mn = jnp.minimum(mn, halves(mn))
        ep = jnp.exp2(p3 - mx[None])
        en = jnp.exp2(mn[None] - p3)
        sp = jnp.sum(ep, axis=0)
        sn = jnp.sum(en, axis=0)
        sp = sp + halves(sp)
        sn = sn + halves(sn)
        rp = 1.0 / sp
        rn = 1.0 / sn
        ep = (ep * rp[None]).reshape(64, TN)
        en = (en * rn[None]).reshape(64, TN)
        return _pk(ep, en)

    def a_layer(extra1=None, extra2=None):
        kvacc[...] = jnp.zeros_like(kvacc)
        ones = jnp.full((8, TN), 0x3F803F80, U32)

        def p1_tile(t, xn_cur, xn_nxt):
            t0 = pl.multiple_of(t * TN, TN)

            def mm(j, part, toks=()):
                return _dot(_b(tie(Wt[j, 32 * part:32 * part + 32, :], toks)), _b(xn_cur[...]))
            seq = [(j, p) for j in range(8) for p in range(3)]
            tn0 = pl.multiple_of(jnp.minimum(t + 1, NT - 1) * TN, TN)
            side = ln_steps(xn_nxt, tn0)
            slots = spread(len(seq) - 2, side)
            if extra1 is not None:
                slots2 = spread(len(seq), extra1(t))
            cur = mm(0, 0)
            pk = None
            pend = []
            lag = [[], []]
            for idx, (j, p) in enumerate(seq):
                nxt = mm(*seq[idx + 1], lag[0]) if idx + 1 < len(seq) else None
                if p == 0:
                    phq[j, :, pl.ds(t0, TN)] = feat(cur)
                elif p == 1:
                    pk = feat(cur)
                else:
                    v1 = _b(jnp.concatenate([_pk(cur[0:32], cur[32:64]), ones], axis=0))
                    kvacc[j] += _dot_nt(v1, _b(pk))
                toks = []
                if idx < len(slots):
                    toks += run_all(slots[idx])
                if extra1 is not None:
                    toks += run_all(slots2[idx])
                lag = [lag[1], toks] if TIE_LAG else [toks, []]
                cur = nxt

        run_all(ln_steps(xn0, 0))

        def p1(i, carry):
            p1_tile(2 * i, xn0, xn1)
            p1_tile(2 * i + 1, xn1, xn0)
            return carry
        with jax.named_scope('A_p1'):
            lax.fori_loop(0, NT // 2, p1, 0)

        mask = ((_iota((80, 128), 0) // 2) % 4) == ((_iota((80, 128), 1) // 2) % 4)

        def o_steps(ob, t0):
            def nd(j):
                kvm = jnp.where(mask, kvacc[j], 0.0).astype(BF16)
                return _dot(kvm, _b(phq[j, :, pl.ds(t0, TN)]))
            st = {}

            def step(j):
                def f():
                    if j == 0:
                        st['cur'] = nd(0)
                    cur = st['cur']
                    if j < 7:
                        st['cur'] = nd(j + 1)
                    rden = 1.0 / (cur[64:72] + 1e-6)
                    o = (cur[0:64].reshape(8, 8, TN) * rden[None]).reshape(64, TN)
                    w = _pk(o[0:32], o[32:64])
                    ob[j * 32:(j + 1) * 32, :] = w
                    return w[24:32, 128:256]
                return f
            return [step(j) for j in range(8)]

        rev_idx = 127 - _iota((8, 128), 1)

        def lnb_steps(t, st):
            t0 = pl.multiple_of(t * TN, TN)

            def s3(b):
                def f():
                    xb = xT[b * 64:(b + 1) * 64, pl.ds(t0, TN)]
                    xn = (xb - st['m']) * st['rs']
                    dk = dskb[b * 64:(b + 1) * 64, :]
                    xT[b * 64:(b + 1) * 64, pl.ds(t0, TN)] = xb + xn * jnp.concatenate([dk, dk], axis=1)
                    w = _pk(xn[:, 0:128], xn[:, 128:256])
                    for r in range(8):
                        wr = w[r * 8:(r + 1) * 8]
                        UB[pl.ds((b * 64 + r * 8) * P + t, 8, stride=P), :] = wr
                        UR[pl.ds((b * 64 + r * 8) * P + t, 8, stride=P), :] = jnp.take_along_axis(wr, rev_idx, axis=1)
                    return w[56:64]
                return f
            return ln_stat_steps(t0, st)[4:] + [s3(b) for b in range(8)]

        def p2_tile(t, ob_cur, ob_nxt, st_prev):
            t0 = pl.multiple_of(t * TN, TN)
            tn0 = pl.multiple_of(jnp.minimum(t + 1, NT - 1) * TN, TN)
            nb = 512 // MB
            sideA = spread(nb, o_steps(ob_nxt, tn0))
            sideB = spread(nb, lnb_steps(t - 1, st_prev) if st_prev is not None else [])
            sideC = spread(nb, extra2(t) if extra2 is not None else [])

            def mm(b, toks=()):
                return _dot(_b(tie(woT[b * MB // 2:(b + 1) * MB // 2, :], toks)), _b(ob_cur[...]))
            cur = mm(0)
            a = None
            lag = [[], []]
            for b in range(nb):
                nxt = mm(b + 1, lag[0]) if b < nb - 1 else None
                xnew = xT[b * MB:(b + 1) * MB, pl.ds(t0, TN)] + cur
                xT[b * MB:(b + 1) * MB, pl.ds(t0, TN)] = xnew
                s = sum8(xnew)
                a = s if a is None else a + s
                toks = run_all(sideA[b]) + run_all(sideB[b]) + run_all(sideC[b])
                if TIE2 == 0:
                    toks = []
                lag = [lag[1], toks] if TIE2 == 2 else [toks, []]
                cur = nxt
            return jnp.sum(a, axis=0, keepdims=True) * (1.0 / D)

        run_all(o_steps(xn0, 0))
        m0 = p2_tile(0, xn0, xn1, None)
        m1 = p2_tile(1, xn1, xn0, {'m': m0})

        def p2(i, m):
            m = p2_tile(2 * i, xn0, xn1, {'m': m})
            return p2_tile(2 * i + 1, xn1, xn0, {'m': m})
        with jax.named_scope('A_p2loop'):
            m7 = lax.fori_loop(1, NT // 2, p2, m1)
        run_all(lnb_steps(NT - 1, {'m': m7}))

    def prep_ssm():
        ldt = jnp.broadcast_to(ldt_ref[...].astype(F32).reshape(1, D), (128, D)).T
        dt = jnp.exp(ldt).astype(BF16).astype(F32)
        dskb[...] = jnp.broadcast_to(dsk_ref[...].astype(F32).reshape(1, D), (128, D)).T
        lr = dt * are_ref[...].astype(F32)
        li = dt * aim_ref[...].astype(F32)
        m = jnp.exp(lr)
        l1r, l1i = m * jnp.cos(li), m * jnp.sin(li)
        lam[0] = l1r
        lam[1] = l1i
        a, b = l1r, l1i
        for k in range(7):
            a, b = a * a - b * b, 2.0 * a * b
            if k == 3:
                l8[0] = a
                l8[1] = b
        mu[0] = a
        mu[1] = b
        dbr = dt * bre_ref[...].astype(F32)
        dbi = dt * bim_ref[...].astype(F32)
        cr, ci = _cmul(cre_ref[...].astype(F32), cim_ref[...].astype(F32), dbr, dbi)
        cc[0] = cr
        cc[1] = ci
        a, b = _cmul(cr, ci, l1r, l1i)
        cl[0] = a
        cl[1] = b

    def bc(ref, i, d):
        return jnp.broadcast_to(ref[i, pl.ds(d, 1), :], (8, 128))

    def gen_steps(g):
        g0 = pl.multiple_of(g * 8, 8)

        def base():
            ar = lam[0, pl.ds(g0, 8), :]
            ai = lam[1, pl.ds(g0, 8), :]
            ar, ai = ar * ar - ai * ai, 2.0 * ar * ai
            pr = jnp.ones((8, 128), F32)
            pi = jnp.zeros((8, 128), F32)
            for r in range(8):
                p0[0, pl.ds(r, 8, stride=P), :] = pr
                p0[1, pl.ds(r, 8, stride=P), :] = pi
                if r == 0:
                    pr, pi = ar, ai
                elif r < 7:
                    pr, pi = _cmul(pr, pi, ar, ai)
        def chan(d8):
            def f():
                d = g0 + d8
                br = bc(l8, 0, d)
                bi = bc(l8, 1, d)
                l1r = bc(lam, 0, d)
                l1i = bc(lam, 1, d)
                qr = p0[0, d8 * P:d8 * P + 8, :]
                qi = p0[1, d8 * P:d8 * P + 8, :]
                wr, wi = [], []
                for k in range(8):
                    if k > 0:
                        qr, qi = _cmul(qr, qi, br, bi)
                    orr, oi = _cmul(qr, qi, l1r, l1i)
                    wr.append(_pk(qr, orr))
                    wi.append(_pk(qi, oi))
                frw = jnp.concatenate(wr, axis=0)
                fiw = jnp.concatenate(wi, axis=0)
                Fc[d, 0:64, :] = frw
                Fc[d, 64:128, :] = fiw
                grb = _b(frw).T
                gib = _b(fiw).T
                Gc[d, 0:64, :] = _u(grb)
                Gc[d, 64:128, :] = _u(gib)
            return f
        return [base] + [chan(d8) for d8 in range(8)]

    def b_layer(first):
        rev_idx = 127 - _iota((8, 128), 1)
        tri = _iota((16, 128), 1) >= _iota((16, 128), 0)
        lane = _iota((8, 128), 1)

        def stage_i(g, sb):
            g0 = pl.multiple_of(g * 8, 8)
            for d8 in range(8):
                d = g0 + d8
                ur = _b(UR[pl.ds(d * P, 8), :])
                sr = _dot(ur, _b(Fc[d, 0:64, :]))
                si = _dot(ur, _b(Fc[d, 64:128, :]))
                for hf in range(2):
                    sb[0, pl.ds(8 * P * hf + d8, 8, stride=P), :] = sr[8 * hf:8 * hf + 8]
                    sb[1, pl.ds(8 * P * hf + d8, 8, stride=P), :] = si[8 * hf:8 * hf + 8]

        def stage_so(g, sb, yb):
            g0 = pl.multiple_of(g * 8, 8)
            mr = mu[0, pl.ds(g0, 8), :]
            mi = mu[1, pl.ds(g0, 8), :]
            cr = cl[0, pl.ds(g0, 8), :]
            ci = cl[1, pl.ds(g0, 8), :]
            zero = jnp.zeros((8, 128), F32)
            hr = hi = None
            prev = None
            for c in range(NC):
                if c == 0:
                    a, b = zero, zero
                else:
                    a, b = _cmul(cr, ci, hr, hi)
                    b = -b
                if c % 2 == 0:
                    prev = (a, b)
                else:
                    hb[0, pl.ds(c // 2, 8, stride=P), :] = pltpu.pack_elementwise([prev[0], a], packed_dtype=BF16)
                    hb[1, pl.ds(c // 2, 8, stride=P), :] = pltpu.pack_elementwise([prev[1], b], packed_dtype=BF16)
                if c < NC - 1:
                    sr = sb[0, c * P:c * P + 8, :]
                    si = sb[1, c * P:c * P + 8, :]
                    if c == 0:
                        hr, hi = sr, si
                    else:
                        a, b = _cmul(mr, mi, hr, hi)
                        hr, hi = a + sr, b + si
            for d8 in range(8):
                d = g0 + d8
                lr = hb[0, d8 * P:d8 * P + 8, :]
                li = hb[1, d8 * P:d8 * P + 8, :]
                if first:
                    cr = jnp.broadcast_to(cc[0, pl.ds(d, 1), :], (8, 128))
                    ci = jnp.broadcast_to(-cc[1, pl.ds(d, 1), :], (8, 128))
                    lr = jnp.concatenate([lr, _pk(cr, cr)], axis=0)
                    li = jnp.concatenate([li, _pk(ci, ci)], axis=0)
                y = _dot(_b(lr), _b(Gc[d, 0:64, :])) + _dot(_b(li), _b(Gc[d, 64:128, :]))
                if first:
                    K0[pl.ds(pl.multiple_of(d * 8, 8), 8), :] = y[16:24]
                for hf in range(2):
                    yb[pl.ds(8 * P * hf + d8, 8, stride=P), :] = y[8 * hf:8 * hf + 8]

        def stage_t(g, yt):
            g0 = pl.multiple_of(g * 8, 8)
            for d8 in range(8):
                d = g0 + d8
                if first:
                    k8 = K0[pl.ds(pl.multiple_of(d * 8, 8), 8), :]
                    kb = jnp.concatenate([k8, k8], axis=0)
                    b0 = _u(jnp.where(tri, pltpu.roll(kb, 0, 1, stride=1, stride_axis=0), 0.0).astype(BF16))
                    rows = [b0]
                    for k in range(1, 8):
                        rows.append(jnp.where(lane >= 16 * k, pltpu.roll(b0, 16 * k, 1), jnp.uint32(0)))
                    tw = jnp.concatenate(rows, axis=0)
                    Tc[d] = tw
                else:
                    tw = Tc[d]
                y = _dot(_b(UB[pl.ds(d * P, 8), :]), _b(tw))
                for hf in range(2):
                    yt[pl.ds(8 * P * hf + d8, 8, stride=P), :] = y[8 * hf:8 * hf + 8]

        def stage_x(g, yb, yt):
            g0 = pl.multiple_of(g * 8, 8)
            for c in range(NC):
                xT[pl.ds(g0, 8), c * C:(c + 1) * C] += yb[c * P:c * P + 8, :] + yt[c * P:c * P + 8, :]

        sbs, ybs, yts = (sb0, sb1), (yb0, yb1), (yt0, yt1)

        def step(g, par, do_i=True, do_x=True, do_t=True):
            if do_i:
                stage_i(g + 1, sbs[1 - par])
            if do_x:
                stage_x(g - 2, ybs[par], yts[par])
            stage_so(g, sbs[par], ybs[par])
            if do_t:
                stage_t(g - 1, yts[1 - par])

        stage_i(0, sb0)
        step(0, 0, do_x=False, do_t=False)
        step(1, 1, do_x=False)

        def out_tile(blk, t):
            b0 = pl.multiple_of(blk * 128, 128)
            t0 = pl.multiple_of(t * 128, 128)
            ostg[blk, pl.ds(t0, 128), :] = xT[pl.ds(b0, 128), pl.ds(t0, 128)].astype(BF16).T

        def out_copy(blk):
            return pltpu.make_async_copy(ostg.at[blk], o_hbm.at[:, pl.ds(blk * 128, 128)], osems.at[blk])

        def grp(i, carry):
            if not first:
                blk = jnp.maximum(i - 4, 0) // 4
                for q in range(4):
                    out_tile(blk, (i % 4) * 4 + q)
            for q in range(2 * UNR):
                step(2 + 2 * UNR * i + q, q % 2)
            if not first:
                @pl.when((i >= 7) & (i % 4 == 3))
                def _():
                    out_copy(blk).start()
            return carry
        with jax.named_scope('B_loop%d' % first):
            lax.fori_loop(0, 60 // (2 * UNR), grp, 0)
        step(62, 0)
        step(63, 1, do_i=False)
        stage_t(63, yt1)
        stage_x(62, yb0, yt0)
        stage_x(63, yb1, yt1)

        if not first:
            for q in range(4):
                out_tile(2, 12 + q)
            out_copy(2).start()
            for q in range(16):
                out_tile(3, q)
            out_copy(3).start()
            for blk in range(4):
                out_copy(blk).wait()

    zero_ref[...] = jnp.zeros((8, 128), U32)
    for cp in prm_copies:
        cp.wait()
    with jax.named_scope('prep_ssm'):
        prep_ssm()
    for cp in w_copies:
        cp.wait()
    with jax.named_scope('prep_w'):
        prep_weights()
    with jax.named_scope('load_x'):
        xs = load_x_steps()
        for q in range(4):
            x_copies[q].wait()
            for s_ in xs[4 * q:4 * q + 4]:
                s_()

    if 'g' in phases:
        def gb(g, carry):
            run_all(gen_steps(g))
            return carry
        lax.fori_loop(0, 64, gb, 0)
    nb_done = [0]
    for ph in phases:
        if ph == 'A':
            with jax.named_scope('A2'):
                a_layer()
        elif ph == 'G':
          with jax.named_scope('A1'):
            a_layer(lambda t: [s for q in range(G1) for s in gen_steps(t * G1 + q)],
                    lambda t: [s for q in range(8 - G1) for s in gen_steps(8 * G1 + t * (8 - G1) + q)])
        elif ph == 'B':
            with jax.named_scope('B%d' % nb_done[0]):
                b_layer(nb_done[0] == 0)
            nb_done[0] += 1


@jax.jit
def pallas_interleave_layers__linear_kernel_hedgehog__ssm_conv_s4__prompt_kernel(
        A_x, A_wqkv, A_w_phi, A_wo, B_u, B_A_re, B_A_im, B_B_re, B_B_im, B_C_re, B_C_im, B_log_dt, B_Dskip):
    del B_u
    x = A_x.reshape(S, D)
    V = pltpu.VMEM
    HBM = pl.BlockSpec(memory_space=pl.ANY)
    VM = pl.BlockSpec(memory_space=pltpu.VMEM)
    scratch = [
        V((S, D), BF16), V((D, 3 * D), BF16), V((D, D), BF16), V((16, 16, 32), BF16), V((6, D, 128), BF16), V((4, S, 128), BF16),
        pltpu.SemaphoreType.DMA((13,)), pltpu.SemaphoreType.DMA((8,)),
        V((D, S), F32),
        V((8, 96, D), U32),
        V((D // 2, D), U32),
        V((8, 64, S), U32),
        V((8, 80, 128), F32),
        V((D, 128, 128), U32),
        V((D, 128, 128), U32),
        V((D, 64, 128), U32),
        V((D * 8, 128), F32),
        V((2, D, 128), F32), V((2, D, 128), F32), V((2, D, 128), F32), V((2, D, 128), F32), V((2, D, 128), F32),
        V((D, 128), F32),
        V((D * P, 128), U32), V((D * P, 128), U32),
        V((2, 8 * P, 128), F32),
        V((2, NC * P, 128), F32), V((2, NC * P, 128), F32),
        V((2, 8 * P, 128), U32),
        V((NC * P, 128), F32), V((NC * P, 128), F32), V((NC * P, 128), F32), V((NC * P, 128), F32),
        V((D // 2, TN), U32), V((D // 2, TN), U32),
        V((8, 128), U32),
    ]
    out = pl.pallas_call(
        functools.partial(_kernel, phases='wpGBAB'),
        out_shape=jax.ShapeDtypeStruct((S, D), BF16),
        in_specs=[HBM, HBM, HBM, HBM, HBM, HBM, HBM, HBM, HBM, HBM, VM, VM],
        out_specs=HBM,
        scratch_shapes=scratch,
        compiler_params=pltpu.CompilerParams(vmem_limit_bytes=120 * 1024 * 1024),
    )(x, A_wqkv, jnp.transpose(A_w_phi, (1, 2, 0)), A_wo, B_A_re, B_A_im, B_B_re, B_B_im, B_C_re, B_C_im,
      B_log_dt, B_Dskip)
    return out.reshape(1, S, D)
```
